```python
import os as _os
_os.environ.setdefault("JAX_PLATFORMS", "cpu")
import jax
import jax.numpy as jnp

def _softmax(x, axis=-1):
    return jax.nn.softmax(x, axis=axis)
def _gelu(x):
    return jax.nn.gelu(x, approximate=True)
def _silu(x):
    return jax.nn.silu(x)
def _sigmoid(x):
    return jax.nn.sigmoid(x)
def _layernorm(x, axis=-1, eps=1e-5):
    m = jnp.mean(x, axis=axis, keepdims=True)
    v = jnp.var(x, axis=axis, keepdims=True)
    return (x - m) / jnp.sqrt(v + eps)
def _scatter_add(tgt, idx, src, axis=0):
    return tgt.at[idx].add(src)
def _segment_sum(src, seg, n):
    return jax.ops.segment_sum(src, seg, n)
class _Rng:
    def __init__(self, key):
        self._k = key
    def _next(self):
        self._k, sub = jax.random.split(self._k)
        return sub
    def normal(self, shape):
        return jax.random.normal(self._next(), shape, dtype=jnp.bfloat16)
    def randint(self, lo, hi, shape):
        return jax.random.randint(self._next(), shape, lo, hi, dtype=jnp.int32)
    def uniform(self, shape, lo=0.0, hi=1.0):
        return jax.random.uniform(self._next(), shape, jnp.bfloat16, lo, hi)
    def permutation(self, n):
        return jax.random.permutation(self._next(), n)


kernel_name = 'gated_mix__linear_attn_block__mixer_token_mlp__prompt'

def setup_inputs():
    _rng = _Rng(jax.random.key(int.from_bytes(__import__("os").urandom(4), "little")))
    _w = (lambda a: (lambda t: t.astype(jnp.bfloat16) if jnp.issubdtype(t.dtype, jnp.floating) else t)(jnp.asarray(a)))
    def _A_setup():
        B, S, D = 1, 2048, 512
        return {
            "x": _w((lambda *s: _rng.normal(s) * 0.05)(B, S, D)),
            "wqkv": _w((lambda *s: _rng.normal(s) * 0.8)(D, 3 * D)),
            "wo": _w((lambda *s: _rng.normal(s) * 0.05)(D, D)),
        }
    _A_in = _A_setup()

    def _B_setup():
        B, S, D, F = 1, 2048, 512, 1792
        return {
            "x": _w((lambda *s: _rng.normal(s) * 0.05)(B, S, D)),
            "w1": _w((lambda *s: _rng.normal(s) * 0.1)(S, F) * (S ** -0.5)),
            "b1": _w((lambda *s: _rng.normal(s) * 0.1)(F) * 0.02),
            "w2": _w((lambda *s: _rng.normal(s) * 0.1)(F, S) * (F ** -0.5)),
            "b2": _w((lambda *s: _rng.normal(s) * 0.1)(S) * 0.02),
        }
    _B_in = _B_setup()

    return {
        "A_x": _A_in["x"],
        "A_wqkv": _A_in["wqkv"],
        "A_wo": _A_in["wo"],
        "B_x": _B_in["x"],
        "B_w1": _B_in["w1"],
        "B_b1": _B_in["b1"],
        "B_w2": _B_in["w2"],
        "B_b2": _B_in["b2"],
        "gate_w": _w((lambda *s: _rng.normal(s) * 0.05)(512) * 16.0),
    }

def reference(A_x, A_wqkv, A_wo, B_x, B_w1, B_b1, B_w2, B_b2, gate_w):
    def _A_ref(x, wqkv, wo):
        B, S, D = x.shape
        H = 32; Dh = D // H
        qkv = (lambda x, *d: x.transpose(*d))((x @ wqkv).reshape(B, S, 3, H, Dh), 2, 0, 3, 1, 4)
        q, k, v = qkv[0], qkv[1], qkv[2]
        phi = lambda t: jnp.where(t > 0, t + 1, jnp.exp(t)) + 1e-6
        pq, pk = phi(q), phi(k)
        kv = jnp.einsum("bhsd,bhse->bhde", pk, v)
        z = jnp.einsum("bhsd->bhd", pk)
        num = jnp.einsum("bhqd,bhde->bhqe", pq, kv)
        den = jnp.einsum("bhqd,bhd->bhq", pq, z)[..., None] + 1e-6
        o = num / den
        return (lambda x, *d: x.transpose(*d))(o, 0, 2, 1, 3).reshape(B, S, D) @ wo

    def _B_ref(x, w1, b1, w2, b2):
        B, S, D = x.shape
        h = _layernorm(x, axis=-1)
        u = jnp.einsum("bsd,sf->bdf", h, w1) + b1
        u = _gelu(u)
        y = jnp.einsum("bdf,fs->bds", u, w2) + b2
        return (lambda x, *d: x.transpose(*d))(y, 0, 2, 1)

    x = A_x
    g = _sigmoid((x * gate_w).sum(-1, keepdims=True))
    a = _A_ref(x, A_wqkv, A_wo)
    b = _B_ref(x, B_w1, B_b1, B_w2, B_b2)
    return g * a + (1 - g) * b
```

```python
import contextlib
import jax
import jax.numpy as jnp
from jax import lax
from jax.experimental import pallas as pl
from jax.experimental.pallas import tpu as pltpu

S, D, F, H = 2048, 512, 1792, 32
DH = D // H
bf = jnp.bfloat16
f32 = jnp.float32
NT = (((1,), (1,)), ((), ()))
NN = (((1,), (0,)), ((), ()))


def _phi(t):
    return jnp.where(t > 0, t + 1.0, jnp.exp(t)) + 1e-6


def _gelu(x):
    c = 0.7978845608028654
    return 0.5 * x * (1.0 + jnp.tanh(c * (x + 0.044715 * (x * x * x))))


def make(CH=(256, 512, 512, 512, 256), XG=(1, 1, 3), Q=(512, 512, 512, 512), C3=(256,) * 8, flags=None, LNR=16, LNB=128,
         pin=6, rawpin=True, scopes=False, semchk=False, WKP=2, rcpmode='nr', UP=(256,) * 7, kvpos=1,
         AP=None, amode='p3', lastsplit=True, lnfirst=True, qfirst=0, midpin=1024):
    assert sum(CH) == S and sum(Q) == S and sum(C3) == S and sum(XG) == len(CH) and sum(UP) == F
    cum = lambda L: [sum(L[:i]) for i in range(len(L) + 1)]
    ch0, q0, c30, up0 = cum(CH), cum(Q), cum(C3), cum(UP)
    n3 = len(C3)
    if AP is None:
        AP = ((2, 512), (3, 512), (4, 512), (5, 512))

    def body(ax_h, wqkv_h, wo_h, bx_h, w1_h, b1_h, w2_h, b2_h, gw_h, out_h,
             x_v, wqkv_v, wo_v, w1_v, w2_v, b1_v, b2_v, gw_v,
             wkT_v, wqT_v, woT_v, hT_v, act_v, mT_v, zb_v, G_v, pk_v, pq_v, g_v, out_v, raw_v, aT_v, pin_v, sems):
        si = [0]

        def dma(src, dst):
            si[0] += 1
            return pltpu.make_async_copy(src, dst, sems.at[si[0] - 1])

        stack = contextlib.ExitStack()

        def scope(name):
            if scopes:
                stack.close()
                if name:
                    stack.enter_context(jax.named_scope(name))

        wr = D // WKP
        c_wk = [dma(wqkv_h.at[pl.ds(i * wr, wr), pl.ds(D, D)], wqkv_v.at[pl.ds(i * wr, wr), pl.ds(D, D)]) for i in range(WKP)]
        xg0 = cum(XG)
        c_xg = []
        for gi in range(len(XG)):
            t0, t1 = ch0[xg0[gi]], ch0[xg0[gi + 1]]
            c_xg.append(dma(ax_h.at[0, pl.ds(t0, t1 - t0), :], x_v.at[pl.ds(t0, t1 - t0), :]))
        c_wq = dma(wqkv_h.at[:, pl.ds(0, D)], wqkv_v.at[:, pl.ds(0, D)])
        c_gw = dma(gw_h, gw_v)
        c_b1 = dma(b1_h, b1_v)
        c_b2 = dma(b2_h, b2_v)
        c_wv = dma(wqkv_h.at[:, pl.ds(2 * D, D)], wqkv_v.at[:, pl.ds(2 * D, D)])
        c_wo = dma(wo_h, wo_v)
        c_w1 = dma(w1_h, w1_v)
        c_w2 = dma(w2_h, w2_v)
        c_pin = dma(gw_h, pin_v)
        for c in c_wk + c_xg + [c_wq, c_gw, c_b1, c_b2, c_wv, c_wo, c_w1, c_w2, c_pin]:
            c.start()

        def k_dot(c):
            t0, n = ch0[c], CH[c]
            kT = lax.dot_general(wkT_v[...], x_v[pl.ds(t0, n), :], NT, preferred_element_type=f32)
            pk = _phi(kT)
            pk_v[:, pl.ds(t0, n)] = pk.astype(bf)
            zs = pk[:, 0:128]
            for j in range(1, n // 128):
                zs = zs + pk[:, j * 128:(j + 1) * 128]
            return zs

        def ln_rows(r0, nr):
            xb = x_v[pl.ds(r0, nr), :].astype(f32)
            m = jnp.mean(xb, axis=1, keepdims=True)
            xm = xb - m
            v = jnp.mean(xm * xm, axis=1, keepdims=True)
            return (xm * lax.rsqrt(v + 1e-5)).astype(bf)

        def ln_part(c):
            for b in range(CH[c] // LNB):
                t0 = ch0[c] + b * LNB
                hb = jnp.concatenate([ln_rows(t0 + r * LNR, LNR) for r in range(LNB // LNR)], axis=0)
                hT_v[:, pl.ds(t0, LNB)] = hb.T

        def g_part(c):
            t0, n = ch0[c], CH[c]
            d = lax.dot_general(pk_v[:, pl.ds(t0, n)], x_v[pl.ds(t0, n), :], NN, preferred_element_type=f32)
            if c == 0:
                G_v[...] = d
            else:
                G_v[...] += d

        def q_part(c):
            t0, n = q0[c], Q[c]
            qT = lax.dot_general(wqT_v[...], x_v[pl.ds(t0, n), :], NT, preferred_element_type=f32)
            g_v[:, pl.ds(t0, n)] = qT[D:D + 8, :]
            pq_v[:, pl.ds(t0, n)] = _phi(qT[0:D, :]).astype(bf)

        def u_part(i):
            f0, nf = up0[i], UP[i]
            u = lax.dot_general(hT_v[...], w1_v[:, pl.ds(f0, nf)], NN, preferred_element_type=f32)
            u = u + b1_v[pl.ds(f0, nf)].astype(f32).reshape(1, nf)
            act_v[:, pl.ds(f0, nf)] = _gelu(u).astype(bf)

        def recip(x):
            r = pl.reciprocal(x, approx=True)
            return r * (2.0 - x * r)

        def pq_norm(t0, n):
            g = jax.nn.sigmoid(g_v[0:1, pl.ds(t0, n)])
            pq = pq_v[:, pl.ds(t0, n)].astype(f32)
            zbb = jnp.concatenate([zb_v[...]] * (n // 128), axis=1)
            den = jnp.sum((pq * zbb).reshape(H, DH, n), axis=1, keepdims=True) + 1e-6
            r = g.reshape(1, 1, n) / den if rcpmode == 'div' else g.reshape(1, 1, n) * recip(den)
            return (pq.reshape(H, DH, n) * r).reshape(D, n).astype(bf)

        def a_part(t0, n):
            return lax.dot_general(mT_v[...], pq_norm(t0, n), NN, preferred_element_type=f32)

        scope('r0')
        for i in range(WKP):
            c_wk[i].wait()
            wkT_v[:, pl.ds(i * wr, wr)] = wqkv_v[pl.ds(i * wr, wr), pl.ds(D, D)].T
        zacc = None
        for gi in range(len(XG)):
            scope(f'r1_wait{gi}')
            c_xg[gi].wait()
            last = gi == len(XG) - 1
            if last:
                c_wq.wait(); c_gw.wait()
            scope(f'r1_{gi}')
            if last:
                wqT_v[pl.ds(0, D), :] = wqkv_v[:, pl.ds(0, D)].T
                wqT_v[pl.ds(D, 16), :] = jnp.broadcast_to(gw_v[...].reshape(1, D), (16, D))
            cs = list(range(xg0[gi], xg0[gi + 1]))
            for c in cs:
                if lnfirst: ln_part(c)
                zs = k_dot(c)
                if not lnfirst: ln_part(c)
                zacc = zs if zacc is None else zacc + zs
                if c > cs[0]: g_part(c - 1)
            if not last:
                g_part(cs[-1])
        q_part(0)
        g_part(len(CH) - 1)
        for c in range(1, len(Q)): q_part(c)
        z = jnp.sum(zacc, axis=1, keepdims=True)
        zb_v[...] = jnp.broadcast_to(z, (D, 128))

        scope('r3_wait')
        for c in (c_w1, c_b1, c_b2, c_wv, c_wo): c.wait()
        scope('r3')
        woT_v[...] = wo_v[...].T
        ri = lax.broadcasted_iota(jnp.int32, (128, 128), 0) // DH
        ci = lax.broadcasted_iota(jnp.int32, (128, 128), 1) // DH
        at = 0
        for i in range(len(UP)):
            u_part(i)
            if i == kvpos - 1:
                kvm = []
                for b in range(D // 128):
                    kv = lax.dot_general(G_v[pl.ds(b * 128, 128), :].astype(bf), wqkv_v[:, pl.ds(2 * D + b * 128, 128)], NN,
                                         preferred_element_type=f32)
                    kvm.append(jnp.where(ri == ci, kv, 0.0).astype(bf))
            if i == kvpos:
                for b in range(D // 128):
                    mT_v[:, pl.ds(b * 128, 128)] = lax.dot_general(
                        woT_v[:, pl.ds(b * 128, 128)], kvm[b], NT, preferred_element_type=f32).astype(bf)
            if amode == 'p2':
                for (after, n) in AP:
                    if after == i:
                        aT_v[:, pl.ds(at, n)] = a_part(at, n)
                        at += n
        assert amode != 'p2' or at == S

        scope('r4_wait')
        c_w2.wait()
        scope('r4')
        c_out = []
        for c in range(n3):
            co = 128 if (lastsplit and c == n3 - 1) else C3[c]
            c_out.append([dma(out_v.at[pl.ds(c30[c] + j * co, co), :], out_h.at[0, pl.ds(c30[c] + j * co, co), :])
                          for j in range(C3[c] // co)])

        def finish(c):
            t0, n = c30[c], C3[c]
            if midpin and c == n3 - 1:
                raw_v[:, pl.ds(0, n)] = lax.dot_general(act_v[:, pl.ds(0, midpin)], w2_v[pl.ds(0, midpin), pl.ds(t0, n)], NN,
                                                        preferred_element_type=f32)
                scope('r5_wait'); c_pin.wait(); scope('r5')
                y = raw_v[:, pl.ds(0, n)] + lax.dot_general(act_v[:, pl.ds(midpin, F - midpin)],
                                                            w2_v[pl.ds(midpin, F - midpin), pl.ds(t0, n)], NN,
                                                            preferred_element_type=f32)
            else:
                y = lax.dot_general(act_v[...], w2_v[:, pl.ds(t0, n)], NN, preferred_element_type=f32)
            aT = aT_v[:, pl.ds(t0, n)] if amode == 'p2' else a_part(t0, n)
            g = jax.nn.sigmoid(g_v[0:1, pl.ds(t0, n)])
            y = y + b2_v[pl.ds(t0, n)].astype(f32).reshape(1, n)
            return aT + (1.0 - g) * y

        def store(c, o):
            co = C3[c] // len(c_out[c])
            for j, cp in enumerate(c_out[c]):
                out_v[pl.ds(c30[c] + j * co, co), :] = o[:, j * co:(j + 1) * co].astype(bf).T
                cp.start()

        for c in range(n3):
            o = finish(c)
            if c == pin and not midpin:
                if rawpin:
                    raw_v[:, pl.ds(0, C3[c])] = o
                    scope('r5_wait'); c_pin.wait(); scope('r5')
                    store(c, raw_v[:, pl.ds(0, C3[c])])
                else:
                    store(c, o)
                    scope('r5_wait'); c_pin.wait(); scope('r5')
            else:
                store(c, o)
        scope('r6_outwait')
        for cc in c_out:
            for cp in cc: cp.wait()
        scope(None)
        assert si[0] == nsem, si[0]

    nsem = 9 + WKP + len(XG) + sum((C3[c] // (128 if lastsplit and c == n3 - 1 else C3[c])) for c in range(n3))
    any_spec = pl.BlockSpec(memory_space=pl.ANY)

    def fn(A_x, A_wqkv, A_wo, B_x, B_w1, B_b1, B_w2, B_b2, gate_w):
        return pl.pallas_call(
            body,
            out_shape=jax.ShapeDtypeStruct((1, S, D), bf),
            in_specs=[any_spec] * 9,
            out_specs=any_spec,
            scratch_shapes=[
                pltpu.VMEM((S, D), bf), pltpu.VMEM((D, 3 * D), bf), pltpu.VMEM((D, D), bf),
                pltpu.VMEM((S, F), bf), pltpu.VMEM((F, S), bf),
                pltpu.VMEM((F,), bf), pltpu.VMEM((S,), bf), pltpu.VMEM((D,), bf),
                pltpu.VMEM((D, D), bf), pltpu.VMEM((D + 16, D), bf), pltpu.VMEM((D, D), bf),
                pltpu.VMEM((D, S), bf), pltpu.VMEM((D, F), bf),
                pltpu.VMEM((D, D), bf), pltpu.VMEM((D, 128), f32), pltpu.VMEM((D, D), f32),
                pltpu.VMEM((D, S), bf), pltpu.VMEM((D, S), bf), pltpu.VMEM((8, S), f32),
                pltpu.VMEM((S, D), bf), pltpu.VMEM((D, max(C3)), f32), pltpu.VMEM((D, S), f32), pltpu.VMEM((D,), bf),
                pltpu.SemaphoreType.DMA((nsem,)),
            ],
            compiler_params=pltpu.CompilerParams(vmem_limit_bytes=110 * 2**20, flags=flags,
                                                 disable_semaphore_checks=not semchk),
        )(A_x, A_wqkv, A_wo, B_x, B_w1, B_b1, B_w2, B_b2, gate_w)
    return fn


_fn = make(midpin=512)


@jax.jit
def pallas_gated_mix__linear_attn_block__mixer_token_mlp__prompt_kernel(
    A_x: jax.Array,
    A_wqkv: jax.Array,
    A_wo: jax.Array,
    B_x: jax.Array,
    B_w1: jax.Array,
    B_b1: jax.Array,
    B_w2: jax.Array,
    B_b2: jax.Array,
    gate_w: jax.Array,
):
    return _fn(A_x, A_wqkv, A_wo, B_x, B_w1, B_b1, B_w2, B_b2, gate_w)
```

```python
import jax
import jax.numpy as jnp
from jax import lax
from jax.experimental import pallas as pl
from jax.experimental.pallas import tpu as pltpu

S, D, F, H = 2048, 512, 1792, 32
DH = D // H
T = 128
bf = jnp.bfloat16
f32 = jnp.float32
NT = (((1,), (1,)), ((), ()))
NN = (((1,), (0,)), ((), ()))

CH = (256, 512, 512, 512, 256)
XG = (1, 1, 3)
QC = (512, 512, 512, 512)
UP = (256,) * 7
OC = (256,) * 8
KPIN = 512


def _cum(sizes):
    return [sum(sizes[:i]) for i in range(len(sizes) + 1)]


def _phi(t):
    return jnp.where(t > 0, t + 1.0, jnp.exp(t)) + 1e-6


def _gelu(x):
    return 0.5 * x * (1.0 + jnp.tanh(0.7978845608028654 * (x + 0.044715 * (x * x * x))))


def _recip(x):
    x = jnp.minimum(x, jnp.finfo(f32).max)
    r = pl.reciprocal(x, approx=True)
    return r * (2.0 - x * r)


def _kernel(x_h, wqkv_h, wo_h, w1_h, b1_h, w2_h, b2_h, gw_h, out_h,
            x_v, wqkv_v, wo_v, w1_v, w2_v, b1_v, b2_v, gw_v,
            wkT_v, wqT_v, woT_v, hT_v, act_v, mT_v, zb_v, G_v, pk_v, pq_v, g_v, out_v, raw_v, pin_v, sems):
    ch0, q0, u0, o0, xg0 = _cum(CH), _cum(QC), _cum(UP), _cum(OC), _cum(XG)
    n_sem = [0]

    def dma(src, dst):
        n_sem[0] += 1
        return pltpu.make_async_copy(src, dst, sems.at[n_sem[0] - 1])

    c_wk = [dma(wqkv_h.at[pl.ds(i * (D // 2), D // 2), pl.ds(D, D)], wqkv_v.at[pl.ds(i * (D // 2), D // 2), pl.ds(D, D)])
            for i in range(2)]
    c_gw = dma(gw_h, gw_v)
    c_x = []
    for gi in range(len(XG)):
        rows = pl.ds(ch0[xg0[gi]], ch0[xg0[gi + 1]] - ch0[xg0[gi]])
        c_x.append(dma(x_h.at[0, rows, :], x_v.at[rows, :]))
    c_wq = dma(wqkv_h.at[:, pl.ds(0, D)], wqkv_v.at[:, pl.ds(0, D)])
    c_b1, c_b2 = dma(b1_h, b1_v), dma(b2_h, b2_v)
    c_wv = dma(wqkv_h.at[:, pl.ds(2 * D, D)], wqkv_v.at[:, pl.ds(2 * D, D)])
    c_wo = dma(wo_h, wo_v)
    c_w1 = dma(w1_h, w1_v)
    c_w2 = dma(w2_h, w2_v)
    c_pin = dma(gw_h, pin_v)
    for c in [c_wk[0], c_gw, c_wk[1]] + c_x + [c_wq, c_b1, c_b2, c_wv, c_wo, c_w1, c_w2, c_pin]:
        c.start()

    def k_part(c):
        tok = pl.ds(ch0[c], CH[c])
        pk = _phi(lax.dot_general(wkT_v[...], x_v[tok, :], NT, preferred_element_type=f32))
        pk_v[:, tok] = pk.astype(bf)
        zs = pk[:, 0:T]
        for j in range(1, CH[c] // T):
            zs = zs + pk[:, j * T:(j + 1) * T]
        return zs

    def ln_part(c, gw):
        for b in range(CH[c] // T):
            t0 = ch0[c] + b * T
            hs, logits = [], []
            for r0 in range(t0, t0 + T, 16):
                xb = x_v[pl.ds(r0, 16), :].astype(f32)
                xm = xb - jnp.mean(xb, axis=1, keepdims=True)
                var = jnp.mean(xm * xm, axis=1, keepdims=True)
                hs.append((xm * lax.rsqrt(var + 1e-5)).astype(bf))
                logits.append(jnp.sum(xb * gw, axis=1, keepdims=True))
            hT_v[:, pl.ds(t0, T)] = jnp.concatenate(hs, axis=0).T
            lg = jnp.concatenate(logits, axis=0)
            g_v[:, pl.ds(t0, T)] = jnp.broadcast_to(lg, (T, T)).T[0:8, :]

    def g_part(c):
        tok = pl.ds(ch0[c], CH[c])
        d = lax.dot_general(pk_v[:, tok], x_v[tok, :], NN, preferred_element_type=f32)
        if c == 0:
            G_v[...] = d
        else:
            G_v[...] += d

    def q_part(c):
        tok = pl.ds(q0[c], QC[c])
        qT = lax.dot_general(wqT_v[...], x_v[tok, :], NT, preferred_element_type=f32)
        pq_v[:, tok] = _phi(qT).astype(bf)

    for i in range(2):
        c_wk[i].wait()
        wkT_v[:, pl.ds(i * (D // 2), D // 2)] = wqkv_v[pl.ds(i * (D // 2), D // 2), pl.ds(D, D)].T
    zacc = gw = None
    for gi in range(len(XG)):
        c_x[gi].wait()
        last = gi == len(XG) - 1
        if gi == 0:
            c_gw.wait()
            gw = gw_v[...].astype(f32).reshape(1, D)
        if last:
            c_wq.wait()
            wqT_v[...] = wqkv_v[:, pl.ds(0, D)].T
        cs = list(range(xg0[gi], xg0[gi + 1]))
        for c in cs:
            ln_part(c, gw)
            zs = k_part(c)
            zacc = zs if zacc is None else zacc + zs
            if c > cs[0]:
                g_part(c - 1)
        if not last:
            g_part(cs[-1])
    q_part(0)
    g_part(len(CH) - 1)
    for c in range(1, len(QC)):
        q_part(c)
    zb_v[...] = jnp.broadcast_to(jnp.sum(zacc, axis=1, keepdims=True), (D, T))

    for c in (c_w1, c_b1, c_b2, c_wv, c_wo):
        c.wait()
    woT_v[...] = wo_v[...].T
    same_head = (lax.broadcasted_iota(jnp.int32, (T, T), 0) // DH) == (lax.broadcasted_iota(jnp.int32, (T, T), 1) // DH)
    kvm = []
    for i in range(len(UP)):
        cols = pl.ds(u0[i], UP[i])
        u = lax.dot_general(hT_v[...], w1_v[:, cols], NN, preferred_element_type=f32)
        act_v[:, cols] = _gelu(u + b1_v[cols].astype(f32).reshape(1, UP[i])).astype(bf)
        if i == 0:
            for b in range(D // T):
                kv = lax.dot_general(G_v[pl.ds(b * T, T), :].astype(bf), wqkv_v[:, pl.ds(2 * D + b * T, T)], NN,
                                     preferred_element_type=f32)
                kvm.append(jnp.where(same_head, kv, 0.0).astype(bf))
        if i == 1:
            for b in range(D // T):
                mT_v[:, pl.ds(b * T, T)] = lax.dot_general(
                    woT_v[:, pl.ds(b * T, T)], kvm[b], NT, preferred_element_type=f32).astype(bf)

    c_w2.wait()
    c_out = []
    for c in range(len(OC)):
        n = T if c == len(OC) - 1 else OC[c]
        c_out.append([dma(out_v.at[pl.ds(o0[c] + j * n, n), :], out_h.at[0, pl.ds(o0[c] + j * n, n), :])
                      for j in range(OC[c] // n)])

    def finish(c):
        n = OC[c]
        tok = pl.ds(o0[c], n)
        if c == len(OC) - 1:
            raw_v[...] = lax.dot_general(act_v[:, pl.ds(0, KPIN)], w2_v[pl.ds(0, KPIN), tok], NN,
                                         preferred_element_type=f32)
            c_pin.wait()
            y = raw_v[...] + lax.dot_general(act_v[:, pl.ds(KPIN, F - KPIN)], w2_v[pl.ds(KPIN, F - KPIN), tok], NN,
                                             preferred_element_type=f32)
        else:
            y = lax.dot_general(act_v[...], w2_v[:, tok], NN, preferred_element_type=f32)
        g = jax.nn.sigmoid(g_v[0:1, tok])
        pq = pq_v[:, tok].astype(f32)
        zb = jnp.concatenate([zb_v[...]] * (n // T), axis=1)
        den = jnp.sum((pq * zb).reshape(H, DH, n), axis=1, keepdims=True) + 1e-6
        pqn = (pq.reshape(H, DH, n) * (g.reshape(1, 1, n) * _recip(den))).reshape(D, n).astype(bf)
        aT = lax.dot_general(mT_v[...], pqn, NN, preferred_element_type=f32)
        o = aT + (1.0 - g) * (y + b2_v[tok].astype(f32).reshape(1, n))
        m = n // len(c_out[c])
        for j, cp in enumerate(c_out[c]):
            out_v[pl.ds(o0[c] + j * m, m), :] = o[:, j * m:(j + 1) * m].astype(bf).T
            cp.start()

    for c in range(len(OC)):
        finish(c)
    for cs in c_out:
        for cp in cs:
            cp.wait()
    assert n_sem[0] == N_SEM, n_sem[0]


N_SEM = 2 + 1 + len(XG) + 9 + (len(OC) - 1) + OC[-1] // T - 1


@jax.jit
def pallas_gated_mix__linear_attn_block__mixer_token_mlp__prompt_kernel(
    A_x: jax.Array,
    A_wqkv: jax.Array,
    A_wo: jax.Array,
    B_x: jax.Array,
    B_w1: jax.Array,
    B_b1: jax.Array,
    B_w2: jax.Array,
    B_b2: jax.Array,
    gate_w: jax.Array,
):
    del B_x
    vmem = pltpu.VMEM
    hbm = pl.BlockSpec(memory_space=pl.ANY)
    return pl.pallas_call(
        _kernel,
        out_shape=jax.ShapeDtypeStruct((1, S, D), bf),
        in_specs=[hbm] * 8,
        out_specs=hbm,
        scratch_shapes=[
            vmem((S, D), bf), vmem((D, 3 * D), bf), vmem((D, D), bf), vmem((S, F), bf), vmem((F, S), bf),
            vmem((F,), bf), vmem((S,), bf), vmem((D,), bf),
            vmem((D, D), bf), vmem((D, D), bf), vmem((D, D), bf), vmem((D, S), bf), vmem((D, F), bf),
            vmem((D, D), bf), vmem((D, T), f32), vmem((D, D), f32), vmem((D, S), bf), vmem((D, S), bf),
            vmem((8, S), f32), vmem((S, D), bf), vmem((D, OC[-1]), f32), vmem((D,), bf),
            pltpu.SemaphoreType.DMA((N_SEM,)),
        ],
        compiler_params=pltpu.CompilerParams(vmem_limit_bytes=110 * 2**20, disable_semaphore_checks=True),
        name="gated_mix_linear_attn_mixer",
    )(A_x, A_wqkv, A_wo, B_w1, B_b1, B_w2, B_b2, gate_w)
```
